```python
import os as _os
_os.environ.setdefault("JAX_PLATFORMS", "cpu")
import jax
import jax.numpy as jnp

def _softmax(x, axis=-1):
    return jax.nn.softmax(x, axis=axis)
def _gelu(x):
    return jax.nn.gelu(x, approximate=True)
def _silu(x):
    return jax.nn.silu(x)
def _sigmoid(x):
    return jax.nn.sigmoid(x)
def _layernorm(x, axis=-1, eps=1e-5):
    m = jnp.mean(x, axis=axis, keepdims=True)
    v = jnp.var(x, axis=axis, keepdims=True)
    return (x - m) / jnp.sqrt(v + eps)
def _scatter_add(tgt, idx, src, axis=0):
    return tgt.at[idx].add(src)
def _segment_sum(src, seg, n):
    return jax.ops.segment_sum(src, seg, n)
class _Rng:
    def __init__(self, key):
        self._k = key
    def _next(self):
        self._k, sub = jax.random.split(self._k)
        return sub
    def normal(self, shape):
        return jax.random.normal(self._next(), shape, dtype=jnp.bfloat16)
    def randint(self, lo, hi, shape):
        return jax.random.randint(self._next(), shape, lo, hi, dtype=jnp.int32)
    def uniform(self, shape, lo=0.0, hi=1.0):
        return jax.random.uniform(self._next(), shape, jnp.bfloat16, lo, hi)
    def permutation(self, n):
        return jax.random.permutation(self._next(), n)


kernel_name = 'concat_heads__gqa_block_cached__mha_block_cached__near_ridge'

def setup_inputs():
    _rng = _Rng(jax.random.key(int.from_bytes(__import__("os").urandom(4), "little")))
    _w = (lambda a: (lambda t: t.astype(jnp.bfloat16) if jnp.issubdtype(t.dtype, jnp.floating) else t)(jnp.asarray(a)))
    def _A_setup():
        B, Sq, D = 16, 32, 512
        Hq, Hkv, Sk, Dh = 32, 8, 512, 128
        assert Hq % Hkv == 0, (Hq, Hkv)
        return {
            "x": _w((lambda *s: _rng.normal(s) * 0.8)(B, Sq, D)),
            "k_cache": _w((lambda *s: _rng.normal(s) * 0.8)(B, Hkv, Sk, Dh)),
            "v_cache": _w((lambda *s: _rng.normal(s) * 0.05)(B, Hkv, Sk, Dh)),
            "wq": _w((lambda *s: _rng.normal(s) * 0.8)(D, Hq * Dh) * (D ** -0.5)),
            "wo": _w((lambda *s: _rng.normal(s) * 0.05)(Hq * Dh, D) * ((Hq * Dh) ** -0.5)),
        }
    _A_in = _A_setup()

    def _B_setup():
        B, Sq, D = 16, 32, 512
        H, Sk, Dh = 32, 512, 128
        return {
            "x": _w((lambda *s: _rng.normal(s) * 0.8)(B, Sq, D)),
            "k_cache": _w((lambda *s: _rng.normal(s) * 0.8)(B, H, Sk, Dh)),
            "v_cache": _w((lambda *s: _rng.normal(s) * 0.05)(B, H, Sk, Dh)),
            "wq": _w((lambda *s: _rng.normal(s) * 0.8)(D, H * Dh) * (D ** -0.5)),
            "wo": _w((lambda *s: _rng.normal(s) * 0.05)(H * Dh, D) * ((H * Dh) ** -0.5)),
        }
    _B_in = _B_setup()

    return {
        "A_x": _A_in["x"],
        "A_k_cache": _A_in["k_cache"],
        "A_v_cache": _A_in["v_cache"],
        "A_wq": _A_in["wq"],
        "A_wo": _A_in["wo"],
        "B_x": _B_in["x"],
        "B_k_cache": _B_in["k_cache"],
        "B_v_cache": _B_in["v_cache"],
        "B_wq": _B_in["wq"],
        "B_wo": _B_in["wo"],
    }

def reference(A_x, A_k_cache, A_v_cache, A_wq, A_wo, B_x, B_k_cache, B_v_cache, B_wq, B_wo):
    def _A_ref(x, k_cache, v_cache, wq, wo):
        B, Sq, D = x.shape
        Hq, Dh = 32, 128
        Hkv = k_cache.shape[1]
        rep = Hq // Hkv
        q = (lambda x, *d: x.transpose(*d))((x @ wq).reshape(B, Sq, Hq, Dh), 0, 2, 1, 3)
        k = jnp.repeat(k_cache, rep, axis=1)
        v = jnp.repeat(v_cache, rep, axis=1)
        scores = jnp.einsum("bhqd,bhkd->bhqk", q, k) * (Dh ** -0.5)
        p = _softmax(scores, axis=-1)
        o = jnp.einsum("bhqk,bhkd->bhqd", p, v)
        return (lambda x, *d: x.transpose(*d))(o, 0, 2, 1, 3).reshape(B, Sq, Hq * Dh) @ wo

    def _B_ref(x, k_cache, v_cache, wq, wo):
        B, Sq, D = x.shape
        H, Dh = 32, 128
        q = (lambda x, *d: x.transpose(*d))((x @ wq).reshape(B, Sq, H, Dh), 0, 2, 1, 3)
        scores = jnp.einsum("bhqd,bhkd->bhqk", q, k_cache) * (Dh ** -0.5)
        p = _softmax(scores, axis=-1)
        o = jnp.einsum("bhqk,bhkd->bhqd", p, v_cache)
        return (lambda x, *d: x.transpose(*d))(o, 0, 2, 1, 3).reshape(B, Sq, H * Dh) @ wo

    a = _A_ref(A_x, A_k_cache, A_v_cache, A_wq, A_wo)
    b = _B_ref(B_x, B_k_cache, B_v_cache, B_wq, B_wo)
    return jnp.concatenate([a, b], axis=-1)
```

```python
import numpy as np
import jax
import jax.numpy as jnp
from jax import lax
import jax.experimental.pallas as pl
import jax.experimental.pallas.tpu as pltpu

B, SQ, D, H, DH, SK, HKV = 16, 32, 512, 32, 128, 512, 8
REP = H // HKV
GW = REP * DH
NG = HKV
NT_DIMS = (((1,), (1,)), ((), ()))
QSCALE = float(DH ** -0.5 * np.log2(np.e))

NB = 8
RB = 16
WR = 32
L = 3
M = NB * SQ
NQ = B // NB
NSTEP = NG * NQ
NCH = 1 + REP
ND = SK // RB
WD = D // WR
WPS = WD // NQ


def _kernel(ax, ak, av, awq, awo, bx, bk, bv, bwq, bwo, out,
            x_buf, wq_buf, wo_buf, k_buf, v_buf, acc, q_buf, o_buf, out_buf,
            x_sem, wq_sem, wo_sem, kv_sem, out_sem):

    def kv_start(step, j):
        g = step // NQ
        b0 = (step % NQ) * NB
        if j == 0:
            ks, vs, h = ak, av, g
        else:
            ks, vs, h = bk, bv, g * REP + (j - 1)
        for r in range(ND):
            for src, dst, p in ((ks, k_buf, 0), (vs, v_buf, 1)):
                pltpu.make_async_copy(src.at[pl.ds(b0, NB), h, pl.ds(r * RB, RB)],
                                      dst.at[j, :, pl.ds(r * RB, RB)],
                                      kv_sem.at[j]).start(priority=p)

    def kv_wait(j):
        pltpu.make_async_copy(k_buf.at[j], k_buf.at[j], kv_sem.at[j]).wait()
        pltpu.make_async_copy(v_buf.at[j], v_buf.at[j], kv_sem.at[j]).wait()

    def wq_start(g, d0, n):
        slot = g % 2
        for i in range(n):
            r0 = pl.multiple_of((d0 + i) * WR, WR)
            for t, src in enumerate((awq, bwq)):
                pltpu.make_async_copy(
                    src.at[pl.ds(r0, WR), pl.ds(pl.multiple_of(g * GW, GW), GW)],
                    wq_buf.at[slot, t, pl.ds(r0, WR)], wq_sem.at[slot]).start(priority=t)

    def wo_start(g, d0, n):
        slot = g % 2
        for i in range(n):
            r0 = pl.multiple_of((d0 + i) * WR, WR)
            for t, src in enumerate((awo, bwo)):
                pltpu.make_async_copy(
                    src.at[pl.ds(pl.multiple_of(g * GW + r0, WR), WR)],
                    wo_buf.at[slot, t, pl.ds(r0, WR)], wo_sem.at[slot]).start(priority=t)

    def w_wait(buf, sem, slot):
        pltpu.make_async_copy(buf.at[slot], buf.at[slot], sem.at[slot]).wait()

    def softmax_num(s):
        p = jnp.exp2(s - jnp.max(s, axis=-1, keepdims=True))
        return p.astype(jnp.bfloat16), jnp.sum(p, axis=-1, keepdims=True)

    def attend(qs, j):
        ps = [softmax_num(lax.dot_general(q, k_buf[j, b], NT_DIMS,
                                          preferred_element_type=jnp.float32))
              for b, q in enumerate(qs)]
        os = []
        for b, (p, l) in enumerate(ps):
            o = jnp.dot(p, v_buf[j, b], preferred_element_type=jnp.float32)
            os.append((o * (1.0 / l)).astype(jnp.bfloat16))
        return os

    def q_proj(t, wslot, row0):
        q = jnp.dot(x_buf[t, pl.ds(row0, M), :], wq_buf[wslot, t],
                    preferred_element_type=jnp.float32)
        return (q * QSCALE).astype(jnp.bfloat16)

    def out_proj(t, wslot, row0, g):
        y = jnp.dot(o_buf[t], wo_buf[wslot, t], preferred_element_type=jnp.float32)

        @pl.when(g == 0)
        def _():
            acc[t, pl.ds(row0, M), :] = y

        @pl.when(g > 0)
        def _():
            acc[t, pl.ds(row0, M), :] += y

    def out_copy(bq):
        return pltpu.make_async_copy(
            out_buf.at[bq], out.at[pl.ds(pl.multiple_of(bq * M, M), M)], out_sem.at[bq])

    for i in range(B * SQ // WR):
        for t, src in enumerate((ax, bx)):
            pltpu.make_async_copy(src.at[pl.ds(i * WR, WR)], x_buf.at[t, pl.ds(i * WR, WR)],
                                  x_sem.at[0]).start(priority=t)
    wq_start(0, 0, WD)
    for c in range(L):
        kv_start(c // NCH, c % NCH)
        if c == 0:
            wo_start(0, 0, WD)
    pltpu.make_async_copy(x_buf, x_buf, x_sem.at[0]).wait()

    def step_fn(step, carry):
        g = step // NQ
        bq = step % NQ
        row0 = pl.multiple_of(bq * M, M)
        wslot = g % 2

        def prefetch(j):
            nstep = step + (j + L) // NCH

            @pl.when(nstep < NSTEP)
            def _():
                kv_start(nstep, (j + L) % NCH)

        def w_prefetch(start):
            @pl.when(g + 1 < NG)
            def _():
                start(g + 1, bq * WPS, WPS)

        prefetch(0)

        @pl.when(bq == 0)
        def _():
            w_wait(wq_buf, wq_sem, wslot)

        qa = q_proj(0, wslot, row0)
        kv_wait(0)
        qs = [jnp.concatenate([qa[b * SQ:(b + 1) * SQ, h * DH:(h + 1) * DH]
                               for h in range(REP)], axis=0) for b in range(NB)]
        os = attend(qs, 0)
        o_buf[0] = jnp.concatenate(
            [jnp.concatenate([o[h * SQ:(h + 1) * SQ] for h in range(REP)], axis=1)
             for o in os], axis=0)

        @pl.when(bq == 0)
        def _():
            w_wait(wo_buf, wo_sem, wslot)

        for h in range(REP):
            prefetch(1 + h)
            if h == 0:
                q_buf[...] = q_proj(1, wslot, row0)
            if h == 1:
                w_prefetch(wq_start)
                out_proj(0, wslot, row0, g)
            if h == 2:
                w_prefetch(wo_start)
            kv_wait(1 + h)
            qs = [q_buf[b * SQ:(b + 1) * SQ, h * DH:(h + 1) * DH] for b in range(NB)]
            o_buf[1, :, h * DH:(h + 1) * DH] = jnp.concatenate(attend(qs, 1 + h), axis=0)
        out_proj(1, wslot, row0, g)

        @pl.when(g == NG - 1)
        def _():
            out_buf[bq, :, 0:D] = acc[0, pl.ds(row0, M), :].astype(jnp.bfloat16)
            out_buf[bq, :, D:2 * D] = acc[1, pl.ds(row0, M), :].astype(jnp.bfloat16)
            out_copy(bq).start()
        return carry

    lax.fori_loop(0, NSTEP, step_fn, 0)
    for bq in range(NQ):
        out_copy(bq).wait()


@jax.jit
def pallas_concat_heads__gqa_block_cached__mha_block_cached__near_ridge_kernel(
    A_x: jax.Array,
    A_k_cache: jax.Array,
    A_v_cache: jax.Array,
    A_wq: jax.Array,
    A_wo: jax.Array,
    B_x: jax.Array,
    B_k_cache: jax.Array,
    B_v_cache: jax.Array,
    B_wq: jax.Array,
    B_wo: jax.Array,
):
    out = pl.pallas_call(
        _kernel,
        in_specs=[pl.BlockSpec(memory_space=pltpu.HBM)] * 10,
        out_specs=pl.BlockSpec(memory_space=pltpu.HBM),
        out_shape=jax.ShapeDtypeStruct((B * SQ, 2 * D), jnp.bfloat16),
        scratch_shapes=[
            pltpu.VMEM((2, B * SQ, D), jnp.bfloat16),
            pltpu.VMEM((2, 2, D, GW), jnp.bfloat16),
            pltpu.VMEM((2, 2, GW, D), jnp.bfloat16),
            pltpu.VMEM((NCH, NB, SK, DH), jnp.bfloat16),
            pltpu.VMEM((NCH, NB, SK, DH), jnp.bfloat16),
            pltpu.VMEM((2, B * SQ, D), jnp.float32),
            pltpu.VMEM((M, GW), jnp.bfloat16),
            pltpu.VMEM((2, M, GW), jnp.bfloat16),
            pltpu.VMEM((NQ, M, 2 * D), jnp.bfloat16),
            pltpu.SemaphoreType.DMA((1,)),
            pltpu.SemaphoreType.DMA((2,)),
            pltpu.SemaphoreType.DMA((2,)),
            pltpu.SemaphoreType.DMA((NCH,)),
            pltpu.SemaphoreType.DMA((NQ,)),
        ],
        compiler_params=pltpu.CompilerParams(vmem_limit_bytes=64 * 1024 * 1024),
        name="gqa_mha_cached_attention",
    )(A_x.reshape(B * SQ, D), A_k_cache, A_v_cache, A_wq, A_wo,
      B_x.reshape(B * SQ, D), B_k_cache, B_v_cache, B_wq, B_wo)
    return out.reshape(B, SQ, 2 * D)
```

```python
import numpy as np
import jax
import jax.numpy as jnp
from jax import lax
import jax.experimental.pallas as pl
import jax.experimental.pallas.tpu as pltpu

B, SQ, D, H, DH, SK, HKV = 16, 32, 512, 32, 128, 512, 8
REP = H // HKV
GW = REP * DH
HD = H * DH
NT_DIMS = (((1,), (1,)), ((), ()))
QSCALE = float(DH ** -0.5 * np.log2(np.e))

NB = 8
M = NB * SQ
NQ = B // NB
RB = 16
ND = SK // RB
LAST = 10
AHEAD = 2
SLOTS = 4
NA = NQ * HKV
NSTEP = NA + NQ * H
XR = 32
WREG, WROWS = 4, 8
WQR = D // (2 * WREG)
WOR = HD // WREG
NWQ = WQR // WROWS * HKV
NWO = WOR // WROWS


def _kernel(ax, ak, av, awq, awo, bx, bk, bv, bwq, bwo, out,
            x_buf, wq_buf, wo_buf, k_buf, v_buf, acc, qa_buf, qb_buf, oa_buf,
            p_buf, r_buf, out_buf, w_sem, k_sem, v_sem, last_sem, out_sem):

    def wait_all(dst, sem):
        pltpu.make_async_copy(dst, dst, sem).wait()

    def kv_start(ks, vs, bq, h, slot):
        def pair(i, sem):
            rows = pl.ds(pl.multiple_of(i * RB, RB), RB)
            pltpu.make_async_copy(ks.at[pl.ds(bq * NB, NB), h, rows], k_buf.at[slot, :, rows],
                                  k_sem.at[slot]).start(priority=0)
            pltpu.make_async_copy(vs.at[pl.ds(bq * NB, NB), h, rows], v_buf.at[slot, :, rows],
                                  sem.at[slot]).start(priority=1)

        lax.fori_loop(0, ND - LAST, lambda i, _: pair(i, v_sem), None, unroll=4)
        lax.fori_loop(ND - LAST, ND, lambda i, _: pair(i, last_sem), None, unroll=4)

    def a_start(n):
        kv_start(ak, av, n // HKV, n % HKV, n % SLOTS)

    def b_start(n):
        kv_start(bk, bv, (n - NA) // H, (n - NA) % H, n % SLOTS)

    def k_wait(slot):
        wait_all(k_buf.at[slot], k_sem.at[slot])

    def v_wait(slot):
        wait_all(v_buf.at[slot, :, pl.ds(0, (ND - LAST) * RB)], v_sem.at[slot])

    def v_last_wait(slot):
        wait_all(v_buf.at[slot, :, pl.ds((ND - LAST) * RB, LAST * RB)], last_sem.at[slot])

    def x_start():
        def pair(i, _):
            rows = pl.ds(pl.multiple_of(i * XR, XR), XR)
            for t, src in enumerate((ax, bx)):
                pltpu.make_async_copy(src.at[rows], x_buf.at[t, rows],
                                      w_sem.at[0]).start(priority=t)

        lax.fori_loop(0, B * SQ // XR, pair, None)

    def wq_start(t, src):
        def pair(i, _):
            rows = pl.ds(pl.multiple_of((i // HKV) * WROWS, WROWS), WROWS)
            cols = pl.ds(pl.multiple_of((i % HKV) * GW, GW), GW)
            for p in (0, 1):
                pltpu.make_async_copy(src.at[:, p, rows, cols], wq_buf.at[t, :, p, rows, cols],
                                      w_sem.at[1 + t]).start(priority=p)

        lax.fori_loop(0, NWQ, pair, None)

    def wo_start(lo, hi):
        def pair(i, _):
            rows = pl.ds(pl.multiple_of(i * WROWS, WROWS), WROWS)
            for t, src in enumerate((awo, bwo)):
                pltpu.make_async_copy(src.at[:, rows], wo_buf.at[t, :, rows],
                                      w_sem.at[3]).start(priority=t)

        lax.fori_loop(lo, hi, pair, None)

    def out_start(t, bq):
        pltpu.make_async_copy(out_buf.at[t, pl.ds(bq * M, M)],
                              out.at[pl.ds(bq * M, M), pl.ds(t * D, D)], out_sem.at[0]).start()

    def q_proj(t, rows, col0, ncols):
        w = wq_buf[t, :, :, :, pl.ds(col0, ncols)].reshape(D, ncols)
        q = jnp.dot(x_buf[t, rows, :], w, preferred_element_type=jnp.float32)
        return (q * QSCALE).astype(jnp.bfloat16)

    def scores(qs, slot):
        for b, q in enumerate(qs):
            n = q.shape[0]
            s = lax.dot_general(q, k_buf[slot, b], NT_DIMS, preferred_element_type=jnp.float32)
            p = jnp.exp2(s - jnp.max(s, axis=-1, keepdims=True))
            p_buf[b * n:(b + 1) * n] = p.astype(jnp.bfloat16)
            r_buf[b * n:(b + 1) * n] = jnp.broadcast_to(
                1.0 / jnp.sum(p, axis=-1, keepdims=True), (n, DH))

    def values(n, slot):
        os = []
        for b in range(NB):
            o = jnp.dot(p_buf[b * n:(b + 1) * n], v_buf[slot, b],
                        preferred_element_type=jnp.float32)
            os.append((o * r_buf[b * n:(b + 1) * n]).astype(jnp.bfloat16))
        return os

    def out_proj(t, rows, h, o):
        wrows = pl.ds(pl.multiple_of((h * DH) % WOR, DH), DH)
        y = jnp.dot(o, wo_buf[t, (h * DH) // WOR, wrows, :], preferred_element_type=jnp.float32)
        y = jnp.where(h == 0, 0.0, acc[t]) + y
        acc[t] = y
        out_buf[t, rows] = y.astype(jnp.bfloat16)

    x_start()
    wq_start(0, awq)
    wq_start(1, bwq)
    acc[...] = jnp.zeros_like(acc)
    wait_all(x_buf, w_sem.at[0])
    wait_all(wq_buf.at[0], w_sem.at[1])
    wo_steps = HKV - AHEAD
    wo_per_step = pl.cdiv(NWO, wo_steps)

    def qa_step(g, _):
        col0 = pl.multiple_of(g * GW, GW)
        qa_buf[:, pl.ds(col0, GW)] = q_proj(0, slice(None), col0, GW)

        @pl.when(g < wo_steps)
        def _():
            wo_start(g * wo_per_step, jnp.minimum((g + 1) * wo_per_step, NWO))

        @pl.when(g >= wo_steps)
        def _():
            a_start(g - wo_steps)

    lax.fori_loop(0, HKV, qa_step, None)

    def a_step(n, _):
        slot = n % SLOTS

        def head_block(b, h):
            return (pl.ds(pl.multiple_of((n // HKV) * M + b * SQ, SQ), SQ),
                    pl.ds(pl.multiple_of((n % HKV) * GW + h * DH, DH), DH))

        k_wait(slot)
        scores([jnp.concatenate([qa_buf[head_block(b, h)] for h in range(REP)], axis=0)
                for b in range(NB)], slot)

        @pl.when(n + AHEAD < NA)
        def _():
            a_start(n + AHEAD)

        @pl.when(n + AHEAD >= NA)
        def _():
            b_start(n + AHEAD)

        v_wait(slot)
        v_last_wait(slot)
        for b, o in enumerate(values(REP * SQ, slot)):
            for h in range(REP):
                oa_buf[head_block(b, h)] = o[h * SQ:(h + 1) * SQ]

    lax.fori_loop(0, NA, a_step, None)
    wait_all(wq_buf.at[1], w_sem.at[2])
    wait_all(wo_buf, w_sem.at[3])

    def prepare(i):
        rows = pl.ds(pl.multiple_of((i // H) * M, M), M)
        col0 = pl.multiple_of((i % H) * DH, DH)
        qb_buf[...] = q_proj(1, rows, col0, DH)
        out_proj(0, rows, i % H, oa_buf[rows, pl.ds(col0, DH)])

    prepare(0)

    def b_step(n, _):
        i = n - NA
        slot = n % SLOTS
        k_wait(slot)
        scores([qb_buf[b * SQ:(b + 1) * SQ] for b in range(NB)], slot)

        @pl.when(n + AHEAD < NSTEP)
        def _():
            b_start(n + AHEAD)

        @pl.when(n + 1 < NSTEP)
        def _():
            prepare(i + 1)

        v_wait(slot)

        @pl.when(n + 1 == NSTEP)
        def _():
            for bq in range(NQ):
                out_start(0, bq)
                if bq + 1 < NQ:
                    out_start(1, bq)

        v_last_wait(slot)
        out_proj(1, pl.ds(pl.multiple_of((i // H) * M, M), M), i % H,
                 jnp.concatenate(values(SQ, slot), axis=0))

    lax.fori_loop(NA, NSTEP, b_step, None)
    out_start(1, NQ - 1)
    wait_all(out_buf, out_sem.at[0])


@jax.jit
def pallas_concat_heads__gqa_block_cached__mha_block_cached__near_ridge_kernel(
    A_x: jax.Array,
    A_k_cache: jax.Array,
    A_v_cache: jax.Array,
    A_wq: jax.Array,
    A_wo: jax.Array,
    B_x: jax.Array,
    B_k_cache: jax.Array,
    B_v_cache: jax.Array,
    B_wq: jax.Array,
    B_wo: jax.Array,
):
    out = pl.pallas_call(
        _kernel,
        in_specs=[pl.BlockSpec(memory_space=pltpu.HBM)] * 10,
        out_specs=pl.BlockSpec(memory_space=pltpu.HBM),
        out_shape=jax.ShapeDtypeStruct((B * SQ, 2 * D), jnp.bfloat16),
        scratch_shapes=[
            pltpu.VMEM((2, B * SQ, D), jnp.bfloat16),
            pltpu.VMEM((2, WREG, 2, WQR, HD), jnp.bfloat16),
            pltpu.VMEM((2, WREG, WOR, D), jnp.bfloat16),
            pltpu.VMEM((SLOTS, NB, SK, DH), jnp.bfloat16),
            pltpu.VMEM((SLOTS, NB, SK, DH), jnp.bfloat16),
            pltpu.VMEM((2, M, D), jnp.float32),
            pltpu.VMEM((B * SQ, HD), jnp.bfloat16),
            pltpu.VMEM((M, DH), jnp.bfloat16),
            pltpu.VMEM((B * SQ, HD), jnp.bfloat16),
            pltpu.VMEM((REP * M, SK), jnp.bfloat16),
            pltpu.VMEM((REP * M, DH), jnp.float32),
            pltpu.VMEM((2, B * SQ, D), jnp.bfloat16),
            pltpu.SemaphoreType.DMA((4,)),
            pltpu.SemaphoreType.DMA((SLOTS,)),
            pltpu.SemaphoreType.DMA((SLOTS,)),
            pltpu.SemaphoreType.DMA((SLOTS,)),
            pltpu.SemaphoreType.DMA((1,)),
        ],
        compiler_params=pltpu.CompilerParams(
            vmem_limit_bytes=64 * 1024 * 1024,
            disable_bounds_checks=True,
        ),
        name="gqa_mha_cached_attention",
    )(A_x.reshape(B * SQ, D), A_k_cache, A_v_cache,
      A_wq.reshape(WREG, 2, WQR, HD), A_wo.reshape(WREG, WOR, D),
      B_x.reshape(B * SQ, D), B_k_cache, B_v_cache,
      B_wq.reshape(WREG, 2, WQR, HD), B_wo.reshape(WREG, WOR, D))
    return out.reshape(B, SQ, 2 * D)
```

```python
import numpy as np
import jax
import jax.numpy as jnp
from jax import lax
import jax.experimental.pallas as pl
import jax.experimental.pallas.tpu as pltpu

B, SQ, D, H, DH, SK, HKV = 16, 32, 512, 32, 128, 512, 8
REP = H // HKV
GW = REP * DH
HD = H * DH
NT_DIMS = (((1,), (1,)), ((), ()))
QSCALE = float(DH ** -0.5 * np.log2(np.e))

NB = 8
M = NB * SQ
NQ = B // NB
NA = NQ * HKV
NSTEP = NA + NQ * H
AHEAD = 2
KSLOTS = AHEAD
VSLOTS = AHEAD + 1
RB = 16
XR = 32
WREG, WROWS = 4, 8
WQR = D // (2 * WREG)
WOR = HD // WREG
WO_STEPS = HKV - AHEAD
WO_PAIRS = WOR // WROWS
WO_PAIRS_PER_STEP = -(-WO_PAIRS // WO_STEPS)


def _kernel(ax, ak, av, awq, awo, bx, bk, bv, bwq, bwo, out,
            x_buf, wq_buf, wo_buf, k_buf, v_buf, acc, qa_buf, qb_buf, oa_buf,
            p_buf, r_buf, out_buf, k_sem, v_sem):
    x_sem, awq_sem, bwq_sem, wo_sem = k_sem.at[0], k_sem.at[1], v_sem.at[0], v_sem.at[AHEAD]
    out_sem = k_sem.at[NSTEP % KSLOTS]

    def wait_all(dst, sem):
        pltpu.make_async_copy(dst, dst, sem).wait()

    def kv_start(ks, vs, bq, h, n):
        kslot, vslot = n % KSLOTS, n % VSLOTS

        def pair(i, _):
            rows = pl.ds(pl.multiple_of(i * RB, RB), RB)
            pltpu.make_async_copy(ks.at[pl.ds(bq * NB, NB), h, rows], k_buf.at[kslot, :, rows],
                                  k_sem.at[kslot]).start(priority=0)
            pltpu.make_async_copy(vs.at[pl.ds(bq * NB, NB), h, rows], v_buf.at[vslot, :, rows],
                                  v_sem.at[vslot]).start(priority=1)

        lax.fori_loop(0, SK // RB, pair, None, unroll=4)

    def a_start(n):
        kv_start(ak, av, n // HKV, n % HKV, n)

    def b_start(n):
        kv_start(bk, bv, (n - NA) // H, (n - NA) % H, n)

    def k_wait(n):
        wait_all(k_buf.at[n % KSLOTS], k_sem.at[n % KSLOTS])

    def v_wait(n):
        wait_all(v_buf.at[n % VSLOTS], v_sem.at[n % VSLOTS])

    def x_start():
        def pair(i, _):
            rows = pl.ds(pl.multiple_of(i * XR, XR), XR)
            for t, src in enumerate((ax, bx)):
                pltpu.make_async_copy(src.at[rows], x_buf.at[t, rows], x_sem).start(priority=t)

        lax.fori_loop(0, B * SQ // XR, pair, None)

    def wq_start(t, src, sem):
        def row_tile(i, _):
            rows = pl.ds(pl.multiple_of(i * WROWS, WROWS), WROWS)
            for g in range(HKV):
                cols = pl.ds(g * GW, GW)
                for p in range(2):
                    pltpu.make_async_copy(src.at[:, p, rows, cols],
                                          wq_buf.at[t, :, p, rows, cols], sem).start(priority=p)

        lax.fori_loop(0, WQR // WROWS, row_tile, None)

    def wo_start(lo, hi):
        def pair(i, _):
            rows = pl.ds(pl.multiple_of(i * WROWS, WROWS), WROWS)
            for t, src in enumerate((awo, bwo)):
                pltpu.make_async_copy(src.at[:, rows], wo_buf.at[t, :, rows],
                                      wo_sem).start(priority=t)

        lax.fori_loop(lo, hi, pair, None)

    out_copies = [
        pltpu.make_async_copy(out_buf.at[t, pl.ds(bq * M, M)],
                              out.at[pl.ds(bq * M, M), pl.ds(t * D, D)], out_sem)
        for bq in range(NQ) for t in range(2)]

    def q_proj(t, rows, cols):
        w = wq_buf[t, :, :, :, cols].reshape(D, cols.size)
        q = jnp.dot(x_buf[t, rows, :], w, preferred_element_type=jnp.float32)
        return (q * QSCALE).astype(jnp.bfloat16)

    def scores(qs, n):
        for b, q in enumerate(qs):
            m = q.shape[0]
            s = lax.dot_general(q, k_buf[n % KSLOTS, b], NT_DIMS,
                                preferred_element_type=jnp.float32)
            p = jnp.exp2(s - jnp.max(s, axis=-1, keepdims=True))
            p_buf[b * m:(b + 1) * m] = p.astype(jnp.bfloat16)
            r_buf[b * m:(b + 1) * m] = jnp.broadcast_to(
                1.0 / jnp.sum(p, axis=-1, keepdims=True), (m, DH))

    def values(m, n):
        os = []
        for b in range(NB):
            o = jnp.dot(p_buf[b * m:(b + 1) * m], v_buf[n % VSLOTS, b],
                        preferred_element_type=jnp.float32)
            os.append((o * r_buf[b * m:(b + 1) * m]).astype(jnp.bfloat16))
        return os

    def out_proj(t, rows, h, o):
        wrows = pl.ds(pl.multiple_of((h * DH) % WOR, DH), DH)
        y = jnp.dot(o, wo_buf[t, (h * DH) // WOR, wrows, :], preferred_element_type=jnp.float32)
        y = jnp.where(h == 0, 0.0, acc[t]) + y
        acc[t] = y
        out_buf[t, rows] = y.astype(jnp.bfloat16)

    x_start()
    wq_start(0, awq, awq_sem)
    wq_start(1, bwq, bwq_sem)
    acc[...] = jnp.zeros_like(acc)
    wait_all(x_buf, x_sem)
    wait_all(wq_buf.at[0], awq_sem)

    def qa_step(g, _):
        cols = pl.ds(pl.multiple_of(g * GW, GW), GW)
        qa_buf[:, cols] = q_proj(0, slice(None), cols)

        @pl.when(g < WO_STEPS)
        def _():
            wo_start(g * WO_PAIRS_PER_STEP,
                     jnp.minimum((g + 1) * WO_PAIRS_PER_STEP, WO_PAIRS))

        @pl.when(g == WO_STEPS)
        def _():
            wait_all(wq_buf.at[1], bwq_sem)

        @pl.when(g >= WO_STEPS)
        def _():
            a_start(g - WO_STEPS)

    lax.fori_loop(0, HKV, qa_step, None)
    wait_all(wo_buf, wo_sem)

    def a_step(n, _):
        def head_block(b, h):
            return (pl.ds(pl.multiple_of((n // HKV) * M + b * SQ, SQ), SQ),
                    pl.ds(pl.multiple_of((n % HKV) * GW + h * DH, DH), DH))

        k_wait(n)
        scores([jnp.concatenate([qa_buf[head_block(b, h)] for h in range(REP)], axis=0)
                for b in range(NB)], n)

        @pl.when(n + AHEAD < NA)
        def _():
            a_start(n + AHEAD)

        @pl.when(n + AHEAD >= NA)
        def _():
            b_start(n + AHEAD)

        v_wait(n)
        for b, o in enumerate(values(REP * SQ, n)):
            for h in range(REP):
                oa_buf[head_block(b, h)] = o[h * SQ:(h + 1) * SQ]

    lax.fori_loop(0, NA, a_step, None)

    def block_rows(i):
        return pl.ds(pl.multiple_of((i // H) * M, M), M)

    def prepare(i):
        cols = pl.ds(pl.multiple_of((i % H) * DH, DH), DH)
        qb_buf[...] = q_proj(1, block_rows(i), cols)
        out_proj(0, block_rows(i), i % H, oa_buf[block_rows(i), cols])

    prepare(0)

    def b_step(n, _):
        i = n - NA
        k_wait(n)
        scores([qb_buf[b * SQ:(b + 1) * SQ] for b in range(NB)], n)

        @pl.when(n + AHEAD < NSTEP)
        def _():
            b_start(n + AHEAD)

        @pl.when(n + 1 < NSTEP)
        def _():
            prepare(i + 1)

        @pl.when(n + 1 == NSTEP)
        def _():
            for copy in out_copies[:-1]:
                copy.start()

        v_wait(n)
        out_proj(1, block_rows(i), i % H, jnp.concatenate(values(SQ, n), axis=0))

    lax.fori_loop(NA, NSTEP, b_step, None)
    out_copies[-1].start()
    for copy in out_copies:
        copy.wait()


@jax.jit
def pallas_concat_heads__gqa_block_cached__mha_block_cached__near_ridge_kernel(
    A_x: jax.Array,
    A_k_cache: jax.Array,
    A_v_cache: jax.Array,
    A_wq: jax.Array,
    A_wo: jax.Array,
    B_x: jax.Array,
    B_k_cache: jax.Array,
    B_v_cache: jax.Array,
    B_wq: jax.Array,
    B_wo: jax.Array,
):
    out = pl.pallas_call(
        _kernel,
        in_specs=[pl.BlockSpec(memory_space=pltpu.HBM)] * 10,
        out_specs=pl.BlockSpec(memory_space=pltpu.HBM),
        out_shape=jax.ShapeDtypeStruct((B * SQ, 2 * D), jnp.bfloat16),
        scratch_shapes=[
            pltpu.VMEM((2, B * SQ, D), jnp.bfloat16),
            pltpu.VMEM((2, WREG, 2, WQR, HD), jnp.bfloat16),
            pltpu.VMEM((2, WREG, WOR, D), jnp.bfloat16),
            pltpu.VMEM((KSLOTS, NB, SK, DH), jnp.bfloat16),
            pltpu.VMEM((VSLOTS, NB, SK, DH), jnp.bfloat16),
            pltpu.VMEM((2, M, D), jnp.float32),
            pltpu.VMEM((B * SQ, HD), jnp.bfloat16),
            pltpu.VMEM((M, DH), jnp.bfloat16),
            pltpu.VMEM((B * SQ, HD), jnp.bfloat16),
            pltpu.VMEM((REP * M, SK), jnp.bfloat16),
            pltpu.VMEM((REP * M, DH), jnp.float32),
            pltpu.VMEM((2, B * SQ, D), jnp.bfloat16),
            pltpu.SemaphoreType.DMA((KSLOTS,)),
            pltpu.SemaphoreType.DMA((VSLOTS,)),
        ],
        compiler_params=pltpu.CompilerParams(
            vmem_limit_bytes=64 * 1024 * 1024,
            disable_bounds_checks=True,
        ),
        name="gqa_mha_cached_attention",
    )(A_x.reshape(B * SQ, D), A_k_cache, A_v_cache,
      A_wq.reshape(WREG, 2, WQR, HD), A_wo.reshape(WREG, WOR, D),
      B_x.reshape(B * SQ, D), B_k_cache, B_v_cache,
      B_wq.reshape(WREG, 2, WQR, HD), B_wo.reshape(WREG, WOR, D))
    return out.reshape(B, SQ, 2 * D)
```

```python
import numpy as np
import jax
import jax.numpy as jnp
from jax import lax
import jax.experimental.pallas as pl
import jax.experimental.pallas.tpu as pltpu

B, SQ, D, H, DH, SK, HKV = 16, 32, 512, 32, 128, 512, 8
REP = H // HKV
GW = REP * DH
HD = H * DH
NT_DIMS = (((1,), (1,)), ((), ()))
QSCALE = float(DH ** -0.5 * np.log2(np.e))

NR = 8
HG = H // HKV
M = NR // HG * SQ
NA = B // NR * HKV
NSTEP = NA + B * HG // NR * HKV
AHEAD = 2
KSLOTS = AHEAD
VSLOTS = AHEAD + 1
RB = 16
XR = 32
WROWS = 8
WQR = D // (2 * HG)
WOR = HD // HG
WO_STEPS = HKV - AHEAD
WO_PAIRS = WOR // WROWS
WO_PAIRS_PER_STEP = -(-WO_PAIRS // WO_STEPS)


def _kernel(ax, ak, av, awq, awo, bx, bk, bv, bwq, bwo, out,
            x_buf, wq_buf, wo_buf, k_buf, v_buf, acc, qa_buf, qb_buf, oa_buf,
            p_buf, r_buf, out_buf, k_sem, v_sem):
    x_sem, awq_sem, bwq_sem, wo_sem = k_sem.at[0], k_sem.at[1], v_sem.at[0], v_sem.at[AHEAD]
    out_sem = k_sem.at[NSTEP % KSLOTS]

    def wait_all(dst, sem):
        pltpu.make_async_copy(dst, dst, sem).wait()

    def kv_start(ks, vs, i, n):
        ranges, h = pl.ds((i // HKV) * NR, NR), i % HKV
        kslot, vslot = n % KSLOTS, n % VSLOTS

        def pair(j, _):
            rows = pl.ds(pl.multiple_of(j * RB, RB), RB)
            pltpu.make_async_copy(ks.at[ranges, h, rows], k_buf.at[kslot, :, rows],
                                  k_sem.at[kslot]).start(priority=0)
            pltpu.make_async_copy(vs.at[ranges, h, rows], v_buf.at[vslot, :, rows],
                                  v_sem.at[vslot]).start(priority=1)

        lax.fori_loop(0, SK // RB, pair, None, unroll=4)

    def a_start(n):
        kv_start(ak, av, n, n)

    def b_start(n):
        kv_start(bk, bv, n - NA, n)

    def k_wait(n):
        wait_all(k_buf.at[n % KSLOTS], k_sem.at[n % KSLOTS])

    def v_wait(n):
        wait_all(v_buf.at[n % VSLOTS], v_sem.at[n % VSLOTS])

    def x_start():
        def pair(i, _):
            rows = pl.ds(pl.multiple_of(i * XR, XR), XR)
            for t, src in enumerate((ax, bx)):
                pltpu.make_async_copy(src.at[rows], x_buf.at[t, rows], x_sem).start(priority=t)

        lax.fori_loop(0, B * SQ // XR, pair, None)

    def wq_start(t, src, sem):
        def row_tile(i, _):
            rows = pl.ds(pl.multiple_of(i * WROWS, WROWS), WROWS)
            for g in range(HKV):
                cols = pl.ds(g * GW, GW)
                for p in range(2):
                    pltpu.make_async_copy(src.at[:, p, rows, cols],
                                          wq_buf.at[t, :, p, rows, cols], sem).start(priority=p)

        lax.fori_loop(0, WQR // WROWS, row_tile, None)

    def wo_start(lo, hi):
        def pair(i, _):
            rows = pl.ds(pl.multiple_of(i * WROWS, WROWS), WROWS)
            for t, src in enumerate((awo, bwo)):
                pltpu.make_async_copy(src.at[:, rows], wo_buf.at[t, :, rows],
                                      wo_sem).start(priority=t)

        lax.fori_loop(lo, hi, pair, None)

    out_copies = [
        pltpu.make_async_copy(out_buf.at[t, rows], out.at[rows, pl.ds(t * D, D)], out_sem)
        for t, rows in ((0, pl.ds(0, B * SQ)), (1, pl.ds(0, B * SQ - M)),
                        (1, pl.ds(B * SQ - M, M)))]

    def q_proj(t, rows, cols):
        w = jnp.concatenate([wq_buf[t, :, :, :, c].reshape(D, c.size) for c in cols], axis=1)
        q = jnp.dot(x_buf[t, rows, :], w, preferred_element_type=jnp.float32)
        return (q * QSCALE).astype(jnp.bfloat16)

    def scores(qs, n):
        for b, q in enumerate(qs):
            m = q.shape[0]
            s = lax.dot_general(q, k_buf[n % KSLOTS, b], NT_DIMS,
                                preferred_element_type=jnp.float32)
            p = jnp.exp2(s - jnp.max(s, axis=-1, keepdims=True))
            p_buf[b * m:(b + 1) * m] = p.astype(jnp.bfloat16)
            r_buf[b * m:(b + 1) * m] = jnp.broadcast_to(
                1.0 / jnp.sum(p, axis=-1, keepdims=True), (m, DH))

    def values(m, n):
        os = []
        for b in range(NR):
            o = jnp.dot(p_buf[b * m:(b + 1) * m], v_buf[n % VSLOTS, b],
                        preferred_element_type=jnp.float32)
            os.append((o * r_buf[b * m:(b + 1) * m]).astype(jnp.bfloat16))
        return os

    def out_proj(t, rows, h, o):
        w = wo_buf[t, :, pl.ds(pl.multiple_of(h * DH, DH), DH), :].reshape(HG * DH, D)
        y = jnp.dot(o, w, preferred_element_type=jnp.float32)
        y = jnp.where(h == 0, 0.0, acc[t]) + y
        acc[t] = y
        out_buf[t, rows] = y.astype(jnp.bfloat16)

    x_start()
    wq_start(0, awq, awq_sem)
    wq_start(1, bwq, bwq_sem)
    acc[...] = jnp.zeros_like(acc)
    wait_all(x_buf, x_sem)
    wait_all(wq_buf.at[0], awq_sem)

    def qa_step(g, _):
        cols = pl.ds(pl.multiple_of(g * GW, GW), GW)
        qa_buf[:, cols] = q_proj(0, slice(None), [cols])

        @pl.when(g < WO_STEPS)
        def _():
            wo_start(g * WO_PAIRS_PER_STEP,
                     jnp.minimum((g + 1) * WO_PAIRS_PER_STEP, WO_PAIRS))

        @pl.when(g == WO_STEPS)
        def _():
            wait_all(wq_buf.at[1], bwq_sem)

        @pl.when(g >= WO_STEPS)
        def _():
            a_start(g - WO_STEPS)

    lax.fori_loop(0, HKV, qa_step, None)
    wait_all(wo_buf, wo_sem)

    def a_step(n, _):
        def head_block(b, h):
            return (pl.ds(pl.multiple_of(((n // HKV) * NR + b) * SQ, SQ), SQ),
                    pl.ds(pl.multiple_of((n % HKV) * GW + h * DH, DH), DH))

        k_wait(n)
        scores([jnp.concatenate([qa_buf[head_block(b, h)] for h in range(REP)], axis=0)
                for b in range(NR)], n)

        @pl.when(n + AHEAD < NA)
        def _():
            a_start(n + AHEAD)

        @pl.when(n + AHEAD >= NA)
        def _():
            b_start(n + AHEAD)

        v_wait(n)
        for b, o in enumerate(values(REP * SQ, n)):
            for h in range(REP):
                oa_buf[head_block(b, h)] = o[h * SQ:(h + 1) * SQ]

    lax.fori_loop(0, NA, a_step, None)

    def block_rows(i):
        return pl.ds(pl.multiple_of((i // HKV) * M, M), M)

    def prepare(i):
        cols = [pl.ds(pl.multiple_of((g * HKV + i % HKV) * DH, DH), DH) for g in range(HG)]
        qb_buf[...] = q_proj(1, block_rows(i), cols)
        out_proj(0, block_rows(i), i % HKV,
                 jnp.concatenate([oa_buf[block_rows(i), c] for c in cols], axis=1))

    prepare(0)

    def b_step(n, _):
        i = n - NA
        k_wait(n)
        scores([qb_buf[b * SQ:(b + 1) * SQ, g * DH:(g + 1) * DH]
                for b in range(NR // HG) for g in range(HG)], n)

        @pl.when(n + AHEAD < NSTEP)
        def _():
            b_start(n + AHEAD)

        @pl.when(n + 1 < NSTEP)
        def _():
            prepare(i + 1)

        @pl.when(n + 1 == NSTEP)
        def _():
            for copy in out_copies[:-1]:
                copy.start()

        v_wait(n)
        os = values(SQ, n)
        out_proj(1, block_rows(i), i % HKV, jnp.concatenate(
            [jnp.concatenate(os[b * HG:(b + 1) * HG], axis=1) for b in range(NR // HG)], axis=0))

    lax.fori_loop(NA, NSTEP, b_step, None)
    out_copies[-1].start()
    for copy in out_copies:
        copy.wait()


@jax.jit
def pallas_concat_heads__gqa_block_cached__mha_block_cached__near_ridge_kernel(
    A_x: jax.Array,
    A_k_cache: jax.Array,
    A_v_cache: jax.Array,
    A_wq: jax.Array,
    A_wo: jax.Array,
    B_x: jax.Array,
    B_k_cache: jax.Array,
    B_v_cache: jax.Array,
    B_wq: jax.Array,
    B_wo: jax.Array,
):
    out = pl.pallas_call(
        _kernel,
        in_specs=[pl.BlockSpec(memory_space=pltpu.HBM)] * 10,
        out_specs=pl.BlockSpec(memory_space=pltpu.HBM),
        out_shape=jax.ShapeDtypeStruct((B * SQ, 2 * D), jnp.bfloat16),
        scratch_shapes=[
            pltpu.VMEM((2, B * SQ, D), jnp.bfloat16),
            pltpu.VMEM((2, HG, 2, WQR, HD), jnp.bfloat16),
            pltpu.VMEM((2, HG, WOR, D), jnp.bfloat16),
            pltpu.VMEM((KSLOTS, NR, SK, DH), jnp.bfloat16),
            pltpu.VMEM((VSLOTS, NR, SK, DH), jnp.bfloat16),
            pltpu.VMEM((2, M, D), jnp.float32),
            pltpu.VMEM((B * SQ, HD), jnp.bfloat16),
            pltpu.VMEM((M, HG * DH), jnp.bfloat16),
            pltpu.VMEM((B * SQ, HD), jnp.bfloat16),
            pltpu.VMEM((NR * REP * SQ, SK), jnp.bfloat16),
            pltpu.VMEM((NR * REP * SQ, DH), jnp.float32),
            pltpu.VMEM((2, B * SQ, D), jnp.bfloat16),
            pltpu.SemaphoreType.DMA((KSLOTS,)),
            pltpu.SemaphoreType.DMA((VSLOTS,)),
        ],
        compiler_params=pltpu.CompilerParams(
            vmem_limit_bytes=64 * 1024 * 1024,
            disable_bounds_checks=True,
        ),
        name="gqa_mha_cached_attention",
    )(A_x.reshape(B * SQ, D), A_k_cache, A_v_cache,
      A_wq.reshape(HG, 2, WQR, HD), A_wo.reshape(HG, WOR, D),
      B_x.reshape(B * SQ, D),
      B_k_cache.reshape(B * HG, HKV, SK, DH), B_v_cache.reshape(B * HG, HKV, SK, DH),
      B_wq.reshape(HG, 2, WQR, HD), B_wo.reshape(HG, WOR, D))
    return out.reshape(B, SQ, 2 * D)
```

```python
import numpy as np
import jax
import jax.numpy as jnp
from jax import lax
import jax.experimental.pallas as pl
import jax.experimental.pallas.tpu as pltpu

B, SQ, D, H, DH, SK, HKV = 16, 32, 512, 32, 128, 512, 8
REP = H // HKV
GW = REP * DH
HD = H * DH
LANES = 128
NT_DIMS = (((1,), (1,)), ((), ()))
QSCALE = float(DH ** -0.5 * np.log2(np.e))

NR = 8
HG = H // HKV
M = NR // HG * SQ
NA = B // NR * HKV
NSTEP = NA + B * HG // NR * HKV
AHEAD = 2
KSLOTS = AHEAD
VSLOTS = AHEAD + 1
RR, RB = 2, 64
XR = 32
WROWS = 8
WQR = D // (2 * HG)
WOR = HD // HG
WO_STEPS = HKV - AHEAD
WO_PAIRS = WOR // WROWS
WO_PAIRS_PER_STEP = -(-WO_PAIRS // WO_STEPS)
OR = 32
OUT = [(t, r + half * B * SQ // 2) for r in range(0, B * SQ // 2, OR)
       for t in range(2) for half in range(2)]
LAST_OUT = [(t, r) for t, r in OUT if t == 1 and r >= B * SQ - M]
EARLY_OUT = [block for block in OUT if block not in LAST_OUT]


def _kernel(ax, ak, av, awq, awo, bx, bk, bv, bwq, bwo, out,
            x_buf, wq_buf, wo_buf, k_buf, v_buf, acc, qa_buf, qb_buf, oa_buf,
            p_buf, l_buf, out_buf, k_sem, v_sem):
    x_sem, awq_sem, bwq_sem, wo_sem = k_sem.at[0], k_sem.at[1], v_sem.at[0], v_sem.at[AHEAD]
    out_sem = k_sem.at[NSTEP % KSLOTS]

    def wait_all(dst, sem):
        pltpu.make_async_copy(dst, dst, sem).wait()

    def kv_start(ks, vs, i, n):
        kslot, vslot = n % KSLOTS, n % VSLOTS

        def row_block(j, _):
            rows = pl.ds(pl.multiple_of(j * RB, RB), RB)
            for r in range(0, NR, RR):
                src = (pl.ds((i // HKV) * NR + r, RR), i % HKV, rows)
                pltpu.make_async_copy(ks.at[src], k_buf.at[kslot, pl.ds(r, RR), rows],
                                      k_sem.at[kslot]).start(priority=0)
                pltpu.make_async_copy(vs.at[src], v_buf.at[vslot, pl.ds(r, RR), rows],
                                      v_sem.at[vslot]).start(priority=1)

        lax.fori_loop(0, SK // RB, row_block, None, unroll=2)

    def a_start(n):
        kv_start(ak, av, n, n)

    def b_start(n):
        kv_start(bk, bv, n - NA, n)

    def k_wait(n):
        wait_all(k_buf.at[n % KSLOTS], k_sem.at[n % KSLOTS])

    def v_wait(n):
        wait_all(v_buf.at[n % VSLOTS], v_sem.at[n % VSLOTS])

    def x_start():
        def pair(i, _):
            rows = pl.ds(pl.multiple_of(i * XR, XR), XR)
            for t, src in enumerate((ax, bx)):
                pltpu.make_async_copy(src.at[rows], x_buf.at[t, rows], x_sem).start(priority=t)

        lax.fori_loop(0, B * SQ // XR, pair, None)

    def wq_start(t, src, sem):
        def row_tile(i, _):
            rows = pl.ds(pl.multiple_of(i * WROWS, WROWS), WROWS)
            for g in range(HKV):
                cols = pl.ds(g * GW, GW)
                for p in range(2):
                    pltpu.make_async_copy(src.at[:, p, rows, cols],
                                          wq_buf.at[t, :, p, rows, cols], sem).start(priority=p)

        lax.fori_loop(0, WQR // WROWS, row_tile, None)

    def wo_start(lo, hi):
        def pair(i, _):
            rows = pl.ds(pl.multiple_of(i * WROWS, WROWS), WROWS)
            for t, src in enumerate((awo, bwo)):
                pltpu.make_async_copy(src.at[:, rows], wo_buf.at[t, :, rows],
                                      wo_sem).start(priority=t)

        lax.fori_loop(lo, hi, pair, None)

    def out_start(blocks):
        for j, (t, r) in enumerate(blocks):
            rows = pl.ds(r, OR)
            pltpu.make_async_copy(out_buf.at[t, rows], out.at[rows, pl.ds(t * D, D)],
                                  out_sem).start(priority=j % 2)

    def q_proj(t, rows, cols):
        w = jnp.concatenate([wq_buf[t, :, :, :, c].reshape(D, c.size) for c in cols], axis=1)
        q = jnp.dot(x_buf[t, rows, :], w, preferred_element_type=jnp.float32)
        return (q * QSCALE).astype(jnp.bfloat16)

    def scores(qs, n):
        for b, q in enumerate(qs):
            m = q.shape[0]
            s = lax.dot_general(q, k_buf[n % KSLOTS, b], NT_DIMS,
                                preferred_element_type=jnp.float32)
            p = jnp.exp2(s - jnp.max(s, axis=-1, keepdims=True))
            p_buf[b * m:(b + 1) * m] = p.astype(jnp.bfloat16)
            l_buf[b * m:(b + 1) * m] = sum(p[:, c:c + LANES] for c in range(0, SK, LANES))

    def values(m, n):
        os = []
        for b in range(NR):
            o = jnp.dot(p_buf[b * m:(b + 1) * m], v_buf[n % VSLOTS, b],
                        preferred_element_type=jnp.float32)
            l = jnp.sum(l_buf[b * m:(b + 1) * m], axis=-1, keepdims=True)
            os.append((o * (1.0 / l)).astype(jnp.bfloat16))
        return os

    def out_proj(t, rows, h, o):
        w = wo_buf[t, :, pl.ds(pl.multiple_of(h * DH, DH), DH), :].reshape(HG * DH, D)
        y = jnp.dot(o, w, preferred_element_type=jnp.float32)
        y = jnp.where(h == 0, 0.0, acc[t]) + y
        acc[t] = y
        out_buf[t, rows] = y.astype(jnp.bfloat16)

    x_start()
    wq_start(0, awq, awq_sem)
    wq_start(1, bwq, bwq_sem)
    acc[...] = jnp.zeros_like(acc)
    wait_all(x_buf, x_sem)
    wait_all(wq_buf.at[0], awq_sem)

    def qa_step(g, _):
        cols = pl.ds(pl.multiple_of(g * GW, GW), GW)
        qa_buf[:, cols] = q_proj(0, slice(None), [cols])

        @pl.when(g < WO_STEPS)
        def _():
            wo_start(g * WO_PAIRS_PER_STEP,
                     jnp.minimum((g + 1) * WO_PAIRS_PER_STEP, WO_PAIRS))

        @pl.when(g == WO_STEPS)
        def _():
            wait_all(wq_buf.at[1], bwq_sem)

        @pl.when(g >= WO_STEPS)
        def _():
            a_start(g - WO_STEPS)

    lax.fori_loop(0, HKV, qa_step, None)
    wait_all(wo_buf, wo_sem)

    def a_step(n, _):
        def head_block(b, h):
            return (pl.ds(pl.multiple_of(((n // HKV) * NR + b) * SQ, SQ), SQ),
                    pl.ds(pl.multiple_of((n % HKV) * GW + h * DH, DH), DH))

        k_wait(n)
        scores([jnp.concatenate([qa_buf[head_block(b, h)] for h in range(REP)], axis=0)
                for b in range(NR)], n)

        @pl.when(n + AHEAD < NA)
        def _():
            a_start(n + AHEAD)

        @pl.when(n + AHEAD >= NA)
        def _():
            b_start(n + AHEAD)

        v_wait(n)
        for b, o in enumerate(values(REP * SQ, n)):
            for h in range(REP):
                oa_buf[head_block(b, h)] = o[h * SQ:(h + 1) * SQ]

    lax.fori_loop(0, NA, a_step, None)

    def block_rows(i):
        return pl.ds(pl.multiple_of((i // HKV) * M, M), M)

    def prepare(i):
        cols = [pl.ds(pl.multiple_of((g * HKV + i % HKV) * DH, DH), DH) for g in range(HG)]
        qb_buf[...] = q_proj(1, block_rows(i), cols)
        out_proj(0, block_rows(i), i % HKV,
                 jnp.concatenate([oa_buf[block_rows(i), c] for c in cols], axis=1))

    prepare(0)

    def b_step(n, _):
        i = n - NA
        k_wait(n)
        scores([qb_buf[b * SQ:(b + 1) * SQ, g * DH:(g + 1) * DH]
                for b in range(NR // HG) for g in range(HG)], n)

        @pl.when(n + AHEAD < NSTEP)
        def _():
            b_start(n + AHEAD)

        @pl.when(n + 1 < NSTEP)
        def _():
            prepare(i + 1)

        @pl.when(n + 1 == NSTEP)
        def _():
            out_start(EARLY_OUT)

        v_wait(n)
        os = values(SQ, n)
        out_proj(1, block_rows(i), i % HKV, jnp.concatenate(
            [jnp.concatenate(os[b * HG:(b + 1) * HG], axis=1) for b in range(NR // HG)], axis=0))

    lax.fori_loop(NA, NSTEP, b_step, None)
    out_start(LAST_OUT)
    wait_all(out, out_sem)


@jax.jit
def pallas_concat_heads__gqa_block_cached__mha_block_cached__near_ridge_kernel(
    A_x: jax.Array,
    A_k_cache: jax.Array,
    A_v_cache: jax.Array,
    A_wq: jax.Array,
    A_wo: jax.Array,
    B_x: jax.Array,
    B_k_cache: jax.Array,
    B_v_cache: jax.Array,
    B_wq: jax.Array,
    B_wo: jax.Array,
):
    out = pl.pallas_call(
        _kernel,
        in_specs=[pl.BlockSpec(memory_space=pltpu.HBM)] * 10,
        out_specs=pl.BlockSpec(memory_space=pltpu.HBM),
        out_shape=jax.ShapeDtypeStruct((B * SQ, 2 * D), jnp.bfloat16),
        scratch_shapes=[
            pltpu.VMEM((2, B * SQ, D), jnp.bfloat16),
            pltpu.VMEM((2, HG, 2, WQR, HD), jnp.bfloat16),
            pltpu.VMEM((2, HG, WOR, D), jnp.bfloat16),
            pltpu.VMEM((KSLOTS, NR, SK, DH), jnp.bfloat16),
            pltpu.VMEM((VSLOTS, NR, SK, DH), jnp.bfloat16),
            pltpu.VMEM((2, M, D), jnp.float32),
            pltpu.VMEM((B * SQ, HD), jnp.bfloat16),
            pltpu.VMEM((M, HG * DH), jnp.bfloat16),
            pltpu.VMEM((B * SQ, HD), jnp.bfloat16),
            pltpu.VMEM((NR * REP * SQ, SK), jnp.bfloat16),
            pltpu.VMEM((NR * REP * SQ, LANES), jnp.float32),
            pltpu.VMEM((2, B * SQ, D), jnp.bfloat16),
            pltpu.SemaphoreType.DMA((KSLOTS,)),
            pltpu.SemaphoreType.DMA((VSLOTS,)),
        ],
        compiler_params=pltpu.CompilerParams(
            vmem_limit_bytes=64 * 1024 * 1024,
            disable_bounds_checks=True,
        ),
        name="gqa_mha_cached_attention",
    )(A_x.reshape(B * SQ, D), A_k_cache, A_v_cache,
      A_wq.reshape(HG, 2, WQR, HD), A_wo.reshape(HG, WOR, D),
      B_x.reshape(B * SQ, D),
      B_k_cache.reshape(B * HG, HKV, SK, DH), B_v_cache.reshape(B * HG, HKV, SK, DH),
      B_wq.reshape(HG, 2, WQR, HD), B_wo.reshape(HG, WOR, D))
    return out.reshape(B, SQ, 2 * D)
```

```python
import numpy as np
import jax
import jax.numpy as jnp
from jax import lax
import jax.experimental.pallas as pl
import jax.experimental.pallas.tpu as pltpu

B, SQ, D, H, DH, SK, HKV = 16, 32, 512, 32, 128, 512, 8
REP = H // HKV
GW = REP * DH
HD = H * DH
LANES = 128
NT_DIMS = (((1,), (1,)), ((), ()))
QSCALE = float(DH ** -0.5 * np.log2(np.e))

NR = 8
HG = H // HKV
M = NR // HG * SQ
NA = B // NR * HKV
NSTEP = NA + B * HG // NR * HKV
AHEAD = 2
KSLOTS = AHEAD
VSLOTS = AHEAD + 1
RR, RB = 2, 64
XR = 32
WQR, WOR = D // HG, HD // HG
WQ_PIECE, WO_PIECE = (8, 1024), 16
OR = 32
OUT = [(t, r + half * B * SQ // 2) for r in range(0, B * SQ // 2, OR)
       for t in range(2) for half in range(2)]
LAST_OUT = [(t, r) for t, r in OUT if t == 1 and r >= B * SQ - M]
EARLY_OUT = [block for block in OUT if block not in LAST_OUT]


def _kernel(ax, ak, av, awq, awo, bx, bk, bv, bwq, bwo, out,
            x_buf, wq_buf, wo_buf, k_buf, v_buf, acc, qa_buf, qb_buf, oa_buf,
            p_buf, l_buf, out_buf, k_sem, v_sem, w_sem):
    x_sem, out_sem = v_sem.at[AHEAD], k_sem.at[NSTEP % KSLOTS]

    def wait_all(dst, sem):
        pltpu.make_async_copy(dst, dst, sem).wait()

    def kv_start(ks, vs, i, n):
        kslot, vslot = n % KSLOTS, n % VSLOTS

        def row_block(j, _):
            rows = pl.ds(pl.multiple_of(j * RB, RB), RB)
            for r in range(0, NR, RR):
                src = (pl.ds((i // HKV) * NR + r, RR), i % HKV, rows)
                pltpu.make_async_copy(ks.at[src], k_buf.at[kslot, pl.ds(r, RR), rows],
                                      k_sem.at[kslot]).start(priority=0)
                pltpu.make_async_copy(vs.at[src], v_buf.at[vslot, pl.ds(r, RR), rows],
                                      v_sem.at[vslot]).start(priority=1)

        lax.fori_loop(0, SK // RB, row_block, None, unroll=2)

    def a_start(n):
        kv_start(ak, av, n, n)

    def b_start(n):
        kv_start(bk, bv, n - NA, n)

    def k_wait(n):
        wait_all(k_buf.at[n % KSLOTS], k_sem.at[n % KSLOTS])

    def v_wait(n):
        wait_all(v_buf.at[n % VSLOTS], v_sem.at[n % VSLOTS])

    def x_start():
        def pair(i, _):
            rows = pl.ds(pl.multiple_of(i * XR, XR), XR)
            for t, src in enumerate((ax, bx)):
                pltpu.make_async_copy(src.at[rows], x_buf.at[t, rows], x_sem).start(priority=t)

        lax.fori_loop(0, B * SQ // XR, pair, None)

    def w_start():
        def piece(i, _):
            nr, nc = WQ_PIECE
            wq_piece = (pl.ds(pl.multiple_of(i // (HD // nc) * nr, nr), nr),
                        pl.ds(pl.multiple_of(i % (HD // nc) * nc, nc), nc))
            wo_piece = (pl.ds(pl.multiple_of(i * WO_PIECE, WO_PIECE), WO_PIECE),)
            for srcs, dst, where, sem in (((awq, bwq), wq_buf, wq_piece, w_sem.at[0]),
                                          ((awo, bwo), wo_buf, wo_piece, w_sem.at[1])):
                for r in range(0, HG, RR):
                    for t, src in enumerate(srcs):
                        pltpu.make_async_copy(src.at[(pl.ds(r, RR), *where)],
                                              dst.at[(t, pl.ds(r, RR), *where)],
                                              sem).start(priority=t)

        lax.fori_loop(0, WOR // WO_PIECE, piece, None)

    def out_start(blocks):
        for j, (t, r) in enumerate(blocks):
            rows = pl.ds(r, OR)
            pltpu.make_async_copy(out_buf.at[t, rows], out.at[rows, pl.ds(t * D, D)],
                                  out_sem).start(priority=j % 2)

    def q_proj(t, rows, cols):
        w = jnp.concatenate([wq_buf[t, :, :, c].reshape(D, c.size) for c in cols], axis=1)
        q = jnp.dot(x_buf[t, rows, :], w, preferred_element_type=jnp.float32)
        return (q * QSCALE).astype(jnp.bfloat16)

    def scores(qs, n):
        for b, q in enumerate(qs):
            m = q.shape[0]
            s = lax.dot_general(q, k_buf[n % KSLOTS, b], NT_DIMS,
                                preferred_element_type=jnp.float32)
            p = jnp.exp2(s - jnp.max(s, axis=-1, keepdims=True))
            p_buf[b * m:(b + 1) * m] = p.astype(jnp.bfloat16)
            l_buf[b * m:(b + 1) * m] = sum(p[:, c:c + LANES] for c in range(0, SK, LANES))

    def values(m, n):
        os = []
        for b in range(NR):
            o = jnp.dot(p_buf[b * m:(b + 1) * m], v_buf[n % VSLOTS, b],
                        preferred_element_type=jnp.float32)
            l = jnp.sum(l_buf[b * m:(b + 1) * m], axis=-1, keepdims=True)
            os.append((o * (1.0 / l)).astype(jnp.bfloat16))
        return os

    def out_proj(t, rows, h, o):
        w = wo_buf[t, :, pl.ds(pl.multiple_of(h * DH, DH), DH), :].reshape(HG * DH, D)
        y = jnp.dot(o, w, preferred_element_type=jnp.float32)
        y = jnp.where(h == 0, 0.0, acc[t]) + y
        acc[t] = y
        out_buf[t, rows] = y.astype(jnp.bfloat16)

    x_start()
    w_start()
    lax.fori_loop(0, AHEAD, lambda n, _: a_start(n), None)
    acc[...] = jnp.zeros_like(acc)
    wait_all(x_buf, x_sem)
    wait_all(wq_buf, w_sem.at[0])
    wait_all(wo_buf, w_sem.at[1])

    def a_queries(n):
        rows = pl.ds(pl.multiple_of((n // HKV) * NR * SQ, NR * SQ), NR * SQ)
        return q_proj(0, rows, [pl.ds(pl.multiple_of((n % HKV) * GW, GW), GW)])

    qa_buf[0] = a_queries(0)

    def a_step(n, _):
        def head_block(b, h):
            return (pl.ds(pl.multiple_of(((n // HKV) * NR + b) * SQ, SQ), SQ),
                    pl.ds(pl.multiple_of((n % HKV) * GW + h * DH, DH), DH))

        k_wait(n)
        scores([jnp.concatenate([qa_buf[n % 2, b * SQ:(b + 1) * SQ, h * DH:(h + 1) * DH]
                                 for h in range(REP)], axis=0) for b in range(NR)], n)
        qa_buf[(n + 1) % 2] = a_queries(jnp.minimum(n + 1, NA - 1))

        @pl.when(n + AHEAD < NA)
        def _():
            a_start(n + AHEAD)

        @pl.when(n + AHEAD >= NA)
        def _():
            b_start(n + AHEAD)

        v_wait(n)
        for b, o in enumerate(values(REP * SQ, n)):
            for h in range(REP):
                oa_buf[head_block(b, h)] = o[h * SQ:(h + 1) * SQ]

    lax.fori_loop(0, NA, a_step, None)

    def block_rows(i):
        return pl.ds(pl.multiple_of((i // HKV) * M, M), M)

    def prepare(i):
        cols = [pl.ds(pl.multiple_of((g * HKV + i % HKV) * DH, DH), DH) for g in range(HG)]
        qb_buf[...] = q_proj(1, block_rows(i), cols)
        out_proj(0, block_rows(i), i % HKV,
                 jnp.concatenate([oa_buf[block_rows(i), c] for c in cols], axis=1))

    prepare(0)

    def b_step(n, _):
        i = n - NA
        k_wait(n)
        scores([qb_buf[b * SQ:(b + 1) * SQ, g * DH:(g + 1) * DH]
                for b in range(NR // HG) for g in range(HG)], n)

        @pl.when(n + AHEAD < NSTEP)
        def _():
            b_start(n + AHEAD)

        @pl.when(n + 1 < NSTEP)
        def _():
            prepare(i + 1)

        @pl.when(n + 1 == NSTEP)
        def _():
            out_start(EARLY_OUT)

        v_wait(n)
        os = values(SQ, n)
        out_proj(1, block_rows(i), i % HKV, jnp.concatenate(
            [jnp.concatenate(os[b * HG:(b + 1) * HG], axis=1) for b in range(NR // HG)], axis=0))

    lax.fori_loop(NA, NSTEP, b_step, None)
    out_start(LAST_OUT)
    wait_all(out, out_sem)


@jax.jit
def pallas_concat_heads__gqa_block_cached__mha_block_cached__near_ridge_kernel(
    A_x: jax.Array,
    A_k_cache: jax.Array,
    A_v_cache: jax.Array,
    A_wq: jax.Array,
    A_wo: jax.Array,
    B_x: jax.Array,
    B_k_cache: jax.Array,
    B_v_cache: jax.Array,
    B_wq: jax.Array,
    B_wo: jax.Array,
):
    out = pl.pallas_call(
        _kernel,
        in_specs=[pl.BlockSpec(memory_space=pltpu.HBM)] * 10,
        out_specs=pl.BlockSpec(memory_space=pltpu.HBM),
        out_shape=jax.ShapeDtypeStruct((B * SQ, 2 * D), jnp.bfloat16),
        scratch_shapes=[
            pltpu.VMEM((2, B * SQ, D), jnp.bfloat16),
            pltpu.VMEM((2, HG, WQR, HD), jnp.bfloat16),
            pltpu.VMEM((2, HG, WOR, D), jnp.bfloat16),
            pltpu.VMEM((KSLOTS, NR, SK, DH), jnp.bfloat16),
            pltpu.VMEM((VSLOTS, NR, SK, DH), jnp.bfloat16),
            pltpu.VMEM((2, M, D), jnp.float32),
            pltpu.VMEM((2, NR * SQ, GW), jnp.bfloat16),
            pltpu.VMEM((M, HG * DH), jnp.bfloat16),
            pltpu.VMEM((B * SQ, HD), jnp.bfloat16),
            pltpu.VMEM((NR * REP * SQ, SK), jnp.bfloat16),
            pltpu.VMEM((NR * REP * SQ, LANES), jnp.float32),
            pltpu.VMEM((2, B * SQ, D), jnp.bfloat16),
            pltpu.SemaphoreType.DMA((KSLOTS,)),
            pltpu.SemaphoreType.DMA((VSLOTS,)),
            pltpu.SemaphoreType.DMA((2,)),
        ],
        compiler_params=pltpu.CompilerParams(
            vmem_limit_bytes=64 * 1024 * 1024,
            disable_bounds_checks=True,
        ),
        name="gqa_mha_cached_attention",
    )(A_x.reshape(B * SQ, D), A_k_cache, A_v_cache,
      A_wq.reshape(HG, WQR, HD), A_wo.reshape(HG, WOR, D),
      B_x.reshape(B * SQ, D),
      B_k_cache.reshape(B * HG, HKV, SK, DH), B_v_cache.reshape(B * HG, HKV, SK, DH),
      B_wq.reshape(HG, WQR, HD), B_wo.reshape(HG, WOR, D))
    return out.reshape(B, SQ, 2 * D)
```

```python
import numpy as np
import jax
import jax.numpy as jnp
from jax import lax
import jax.experimental.pallas as pl
import jax.experimental.pallas.tpu as pltpu

B, SQ, D, H, DH, SK, HKV = 16, 32, 512, 32, 128, 512, 8
REP = H // HKV
GW = REP * DH
HD = H * DH
LANES = 128
NT_DIMS = (((1,), (1,)), ((), ()))
QSCALE = float(DH ** -0.5 * np.log2(np.e))

NR = 8
HG = H // HKV
M = NR // HG * SQ
NA = B // NR * HKV
NSTEP = NA + B * HG // NR * HKV
AHEAD = 2
KSLOTS = AHEAD
VSLOTS = AHEAD + 1
RR, RB = 2, 64
XR = 32
WQR, WOR = D // HG, HD // HG
WQ_PIECE, WO_PIECE = (8, 1024), 16
OR = 32
OUT = [(t, r + half * B * SQ // 2) for r in range(0, B * SQ // 2, OR)
       for t in range(2) for half in range(2)]
LAST_OUT = [(t, r) for t, r in OUT if t == 1 and r >= B * SQ - M]
EARLY_OUT = [block for block in OUT if block not in LAST_OUT]


def _kernel(ax, ak, av, awq, awo, bx, bk, bv, bwq, bwo, out,
            x_buf, wq_buf, wo_buf, k_buf, v_buf, acc, qa_buf, qb_buf, oa_buf,
            p_buf, l_buf, out_buf, k_sem, v_sem, w_sem):
    x_sem, out_sem = v_sem.at[AHEAD], k_sem.at[NSTEP % KSLOTS]

    def wait_all(dst, sem):
        pltpu.make_async_copy(dst, dst, sem).wait()

    def kv_start(ks, vs, i, n):
        kslot, vslot = n % KSLOTS, n % VSLOTS

        def row_block(j, _):
            rows = pl.ds(pl.multiple_of(j * RB, RB), RB)
            for r in range(0, NR, RR):
                src = (pl.ds((i // HKV) * NR + r, RR), i % HKV, rows)
                pltpu.make_async_copy(ks.at[src], k_buf.at[kslot, pl.ds(r, RR), rows],
                                      k_sem.at[kslot]).start(priority=0)
                pltpu.make_async_copy(vs.at[src], v_buf.at[vslot, pl.ds(r, RR), rows],
                                      v_sem.at[vslot]).start(priority=1)

        lax.fori_loop(0, SK // RB, row_block, None, unroll=2)

    def a_start(n):
        kv_start(ak, av, n, n)

    def b_start(n):
        kv_start(bk, bv, n - NA, n)

    def k_wait(n):
        wait_all(k_buf.at[n % KSLOTS], k_sem.at[n % KSLOTS])

    def v_wait(n):
        wait_all(v_buf.at[n % VSLOTS], v_sem.at[n % VSLOTS])

    def x_start():
        def pair(i, _):
            rows = pl.ds(pl.multiple_of(i * XR, XR), XR)
            for t, src in enumerate((ax, bx)):
                pltpu.make_async_copy(src.at[rows], x_buf.at[t, rows], x_sem).start(priority=t)

        lax.fori_loop(0, B * SQ // XR, pair, None)

    def w_start():
        def piece(i, _):
            nr, nc = WQ_PIECE
            wq_piece = (pl.ds(pl.multiple_of(i // (HD // nc) * nr, nr), nr),
                        pl.ds(pl.multiple_of(i % (HD // nc) * nc, nc), nc))
            wo_piece = (pl.ds(pl.multiple_of(i * WO_PIECE, WO_PIECE), WO_PIECE),)
            for srcs, dst, where, sem in (((awq, bwq), wq_buf, wq_piece, w_sem.at[0]),
                                          ((awo, bwo), wo_buf, wo_piece, w_sem.at[1])):
                for r in range(0, HG, RR):
                    for t, src in enumerate(srcs):
                        pltpu.make_async_copy(src.at[(pl.ds(r, RR), *where)],
                                              dst.at[(t, pl.ds(r, RR), *where)],
                                              sem).start(priority=t)

        lax.fori_loop(0, WOR // WO_PIECE, piece, None)

    def out_start(blocks):
        for j, (t, r) in enumerate(blocks):
            rows = pl.ds(r, OR)
            pltpu.make_async_copy(out_buf.at[t, rows], out.at[rows, pl.ds(t * D, D)],
                                  out_sem).start(priority=j % 2)

    def q_proj(t, rows, cols):
        w = jnp.concatenate([wq_buf[t, :, :, c].reshape(D, c.size) for c in cols], axis=1)
        q = jnp.dot(x_buf[t, rows, :], w, preferred_element_type=jnp.float32)
        return (q * QSCALE).astype(jnp.bfloat16)

    def scores(qs, n):
        for b, q in enumerate(qs):
            m = q.shape[0]
            s = lax.dot_general(q, k_buf[n % KSLOTS, b], NT_DIMS,
                                preferred_element_type=jnp.float32)
            p = jnp.exp2(s - jnp.max(s, axis=-1, keepdims=True))
            p_buf[b * m:(b + 1) * m] = p.astype(jnp.bfloat16)
            l_buf[b * m:(b + 1) * m] = sum(p[:, c:c + LANES] for c in range(0, SK, LANES))

    def values(m, n):
        os = []
        for b in range(NR):
            o = jnp.dot(p_buf[b * m:(b + 1) * m], v_buf[n % VSLOTS, b],
                        preferred_element_type=jnp.float32)
            l = jnp.sum(l_buf[b * m:(b + 1) * m], axis=-1, keepdims=True)
            os.append((o * (1.0 / l)).astype(jnp.bfloat16))
        return os

    def out_proj(t, rows, h, o):
        w = wo_buf[t, :, pl.ds(pl.multiple_of(h * DH, DH), DH), :].reshape(HG * DH, D)
        y = jnp.dot(o, w, preferred_element_type=jnp.float32)
        y = jnp.where(h == 0, 0.0, acc[t]) + y
        acc[t] = y
        out_buf[t, rows] = y.astype(jnp.bfloat16)

    x_start()
    w_start()
    lax.fori_loop(0, AHEAD, lambda n, _: a_start(n), None)
    acc[...] = jnp.zeros_like(acc)
    wait_all(x_buf, x_sem)
    wait_all(wq_buf, w_sem.at[0])
    wait_all(wo_buf, w_sem.at[1])

    def a_queries(n):
        rows = pl.ds(pl.multiple_of((n // HKV) * NR * SQ, NR * SQ), NR * SQ)
        return q_proj(0, rows, [pl.ds(pl.multiple_of((n % HKV) * GW, GW), GW)])

    qa_buf[0] = a_queries(0)

    def a_step(n, _):
        k_wait(n)
        scores([jnp.concatenate([qa_buf[n % 2, b * SQ:(b + 1) * SQ, h * DH:(h + 1) * DH]
                                 for h in range(REP)], axis=0) for b in range(NR)], n)
        qa_buf[(n + 1) % 2] = a_queries(jnp.minimum(n + 1, NA - 1))

        @pl.when(n + AHEAD < NA)
        def _():
            a_start(n + AHEAD)

        @pl.when(n + AHEAD >= NA)
        def _():
            b_start(n + AHEAD)

        v_wait(n)
        for b, o in enumerate(values(REP * SQ, n)):
            rows = pl.ds(pl.multiple_of(((n // HKV) * NR + b) * SQ, SQ), SQ)
            for h in range(REP):
                cols = pl.ds(pl.multiple_of((n % HKV) * GW + h * DH, DH), DH)
                oa_buf[rows, cols] = o[h * SQ:(h + 1) * SQ]

    lax.fori_loop(0, NA, a_step, None)

    def block_rows(i):
        return pl.ds(pl.multiple_of((i // HKV) * M, M), M)

    def prepare(i):
        cols = [pl.ds(pl.multiple_of((g * HKV + i % HKV) * DH, DH), DH) for g in range(HG)]
        qb_buf[...] = q_proj(1, block_rows(i), cols)
        out_proj(0, block_rows(i), i % HKV,
                 jnp.concatenate([oa_buf[block_rows(i), c] for c in cols], axis=1))

    prepare(0)

    def b_step(n, _):
        i = n - NA
        k_wait(n)
        scores([qb_buf[b * SQ:(b + 1) * SQ, g * DH:(g + 1) * DH]
                for b in range(NR // HG) for g in range(HG)], n)

        @pl.when(n + AHEAD < NSTEP)
        def _():
            b_start(n + AHEAD)

        @pl.when(n + 1 < NSTEP)
        def _():
            prepare(i + 1)

        @pl.when(n + 1 == NSTEP)
        def _():
            out_start(EARLY_OUT)

        v_wait(n)
        os = values(SQ, n)
        out_proj(1, block_rows(i), i % HKV, jnp.concatenate(
            [jnp.concatenate(os[b * HG:(b + 1) * HG], axis=1) for b in range(NR // HG)], axis=0))

    lax.fori_loop(NA, NSTEP, b_step, None)
    out_start(LAST_OUT)
    wait_all(out, out_sem)


@jax.jit
def pallas_concat_heads__gqa_block_cached__mha_block_cached__near_ridge_kernel(
    A_x: jax.Array,
    A_k_cache: jax.Array,
    A_v_cache: jax.Array,
    A_wq: jax.Array,
    A_wo: jax.Array,
    B_x: jax.Array,
    B_k_cache: jax.Array,
    B_v_cache: jax.Array,
    B_wq: jax.Array,
    B_wo: jax.Array,
):
    out = pl.pallas_call(
        _kernel,
        in_specs=[pl.BlockSpec(memory_space=pltpu.HBM)] * 10,
        out_specs=pl.BlockSpec(memory_space=pltpu.HBM),
        out_shape=jax.ShapeDtypeStruct((B * SQ, 2 * D), jnp.bfloat16),
        scratch_shapes=[
            pltpu.VMEM((2, B * SQ, D), jnp.bfloat16),
            pltpu.VMEM((2, HG, WQR, HD), jnp.bfloat16),
            pltpu.VMEM((2, HG, WOR, D), jnp.bfloat16),
            pltpu.VMEM((KSLOTS, NR, SK, DH), jnp.bfloat16),
            pltpu.VMEM((VSLOTS, NR, SK, DH), jnp.bfloat16),
            pltpu.VMEM((2, M, D), jnp.float32),
            pltpu.VMEM((2, NR * SQ, GW), jnp.bfloat16),
            pltpu.VMEM((M, HG * DH), jnp.bfloat16),
            pltpu.VMEM((B * SQ, HD), jnp.bfloat16),
            pltpu.VMEM((NR * REP * SQ, SK), jnp.bfloat16),
            pltpu.VMEM((NR * REP * SQ, LANES), jnp.float32),
            pltpu.VMEM((2, B * SQ, D), jnp.bfloat16),
            pltpu.SemaphoreType.DMA((KSLOTS,)),
            pltpu.SemaphoreType.DMA((VSLOTS,)),
            pltpu.SemaphoreType.DMA((2,)),
        ],
        compiler_params=pltpu.CompilerParams(
            vmem_limit_bytes=64 * 1024 * 1024,
            disable_bounds_checks=True,
        ),
        name="gqa_mha_cached_attention",
    )(A_x.reshape(B * SQ, D), A_k_cache, A_v_cache,
      A_wq.reshape(HG, WQR, HD), A_wo.reshape(HG, WOR, D),
      B_x.reshape(B * SQ, D),
      B_k_cache.reshape(B * HG, HKV, SK, DH), B_v_cache.reshape(B * HG, HKV, SK, DH),
      B_wq.reshape(HG, WQR, HD), B_wo.reshape(HG, WOR, D))
    return out.reshape(B, SQ, 2 * D)
```
